```python
import os as _os
_os.environ.setdefault("JAX_PLATFORMS", "cpu")
import jax
import jax.numpy as jnp

def _softmax(x, axis=-1):
    return jax.nn.softmax(x, axis=axis)
def _gelu(x):
    return jax.nn.gelu(x, approximate=True)
def _silu(x):
    return jax.nn.silu(x)
def _sigmoid(x):
    return jax.nn.sigmoid(x)
def _layernorm(x, axis=-1, eps=1e-5):
    m = jnp.mean(x, axis=axis, keepdims=True)
    v = jnp.var(x, axis=axis, keepdims=True)
    return (x - m) / jnp.sqrt(v + eps)
def _scatter_add(tgt, idx, src, axis=0):
    return tgt.at[idx].add(src)
def _segment_sum(src, seg, n):
    return jax.ops.segment_sum(src, seg, n)
class _Rng:
    def __init__(self, key):
        self._k = key
    def _next(self):
        self._k, sub = jax.random.split(self._k)
        return sub
    def normal(self, shape):
        return jax.random.normal(self._next(), shape, dtype=jnp.bfloat16)
    def randint(self, lo, hi, shape):
        return jax.random.randint(self._next(), shape, lo, hi, dtype=jnp.int32)
    def uniform(self, shape, lo=0.0, hi=1.0):
        return jax.random.uniform(self._next(), shape, jnp.bfloat16, lo, hi)
    def permutation(self, n):
        return jax.random.permutation(self._next(), n)


kernel_name = 'gated_mix__gqa_block_cached__dense_activation_squared_relu__decode'

def setup_inputs():
    _rng = _Rng(jax.random.key(int.from_bytes(__import__("os").urandom(4), "little")))
    _w = (lambda a: (lambda t: t.astype(jnp.bfloat16) if jnp.issubdtype(t.dtype, jnp.floating) else t)(jnp.asarray(a)))
    def _A_setup():
        B, Sq, D = 4, 1, 512
        Hq, Hkv, Sk, Dh = 32, 8, 4096, 128
        assert Hq % Hkv == 0, (Hq, Hkv)
        return {
            "x": _w((lambda *s: _rng.normal(s) * 0.05)(B, Sq, D)),
            "k_cache": _w((lambda *s: _rng.normal(s) * 3.2)(B, Hkv, Sk, Dh)),
            "v_cache": _w((lambda *s: _rng.normal(s) * 1.6)(B, Hkv, Sk, Dh)),
            "wq": _w((lambda *s: _rng.normal(s) * 3.2)(D, Hq * Dh) * (D ** -0.5)),
            "wo": _w((lambda *s: _rng.normal(s) * 1.6)(Hq * Dh, D) * ((Hq * Dh) ** -0.5)),
        }
    _A_in = _A_setup()

    def _B_setup():
        B, S, D, F = 4, 1, 512, 1792
        return {
            "x": _w((lambda *s: _rng.normal(s) * 0.05)(B, S, D)),
            "w1": _w((lambda *s: _rng.normal(s) * 0.1)(D, F)),
            "b1": _w((lambda *s: _rng.normal(s) * 0.05)(F)),
            "w2": _w((lambda *s: _rng.normal(s) * 0.05)(F, D)),
            "b2": _w((lambda *s: _rng.normal(s) * 0.05)(D)),
        }
    _B_in = _B_setup()

    return {
        "A_x": _A_in["x"],
        "A_k_cache": _A_in["k_cache"],
        "A_v_cache": _A_in["v_cache"],
        "A_wq": _A_in["wq"],
        "A_wo": _A_in["wo"],
        "B_x": _B_in["x"],
        "B_w1": _B_in["w1"],
        "B_b1": _B_in["b1"],
        "B_w2": _B_in["w2"],
        "B_b2": _B_in["b2"],
        "gate_w": _w((lambda *s: _rng.normal(s) * 0.05)(512) * 16.0),
    }

def reference(A_x, A_k_cache, A_v_cache, A_wq, A_wo, B_x, B_w1, B_b1, B_w2, B_b2, gate_w):
    def _A_ref(x, k_cache, v_cache, wq, wo):
        B, Sq, D = x.shape
        Hq, Dh = 32, 128
        Hkv = k_cache.shape[1]
        rep = Hq // Hkv
        q = (lambda x, *d: x.transpose(*d))((x @ wq).reshape(B, Sq, Hq, Dh), 0, 2, 1, 3)
        k = jnp.repeat(k_cache, rep, axis=1)
        v = jnp.repeat(v_cache, rep, axis=1)
        scores = jnp.einsum("bhqd,bhkd->bhqk", q, k) * (Dh ** -0.5)
        p = _softmax(scores, axis=-1)
        o = jnp.einsum("bhqk,bhkd->bhqd", p, v)
        return (lambda x, *d: x.transpose(*d))(o, 0, 2, 1, 3).reshape(B, Sq, Hq * Dh) @ wo

    def _B_ref(x, w1, b1, w2, b2):
        h = jnp.einsum("bsd,df->bsf", x, w1) + b1
        zero = jnp.zeros_like(h)
        r = jnp.where(h > zero, h, zero)
        h = r * r
        out = jnp.einsum("bsf,fd->bsd", h, w2) + b2
        return out

    x = A_x
    g = _sigmoid((x * gate_w).sum(-1, keepdims=True))
    a = _A_ref(x, A_k_cache, A_v_cache, A_wq, A_wo)
    b = _B_ref(x, B_w1, B_b1, B_w2, B_b2)
    return g * a + (1 - g) * b
```

```python
import functools

import jax
import jax.numpy as jnp
import jax.experimental.pallas as pl
import jax.experimental.pallas.tpu as pltpu
from jax import lax

_ROWS = 8
_F_CHUNK = 128


def _kernel(x_ref, k_ref, v_ref, wq_ref, wo_ref, w1_ref, b1_ref, w2_ref, b2_ref,
            gw_ref, o_ref, q_scr, o_scr, acc_scr, mlp_scr,
            *, n_batch, rep, dh, n_fchunks):
    h = pl.program_id(0)
    b = pl.program_id(1)
    step = h * n_batch + b
    n_steps = pl.num_programs(0) * pl.num_programs(1)
    scale = dh ** -0.5

    x = x_ref[...]

    @pl.when(step == 0)
    def _init():
        acc_scr[...] = jnp.zeros_like(acc_scr)
        mlp_scr[...] = jnp.zeros_like(mlp_scr)
        q_scr[...] = jnp.zeros_like(q_scr)
        o_scr[...] = jnp.zeros_like(o_scr)

    @pl.when(b == 0)
    def _qproj():
        for j in range(rep):
            qj = jnp.dot(x, wq_ref[:, j * dh:(j + 1) * dh],
                         preferred_element_type=jnp.float32)
            for bb in range(n_batch):
                q_scr[bb, j:j + 1, :] = qj[bb:bb + 1, :]

    @pl.when(step < n_fchunks)
    def _mlp():
        hid = jnp.dot(x, w1_ref[...], preferred_element_type=jnp.float32)
        hid = hid + b1_ref[...].astype(jnp.float32)
        r = jnp.maximum(hid, 0.0)
        hh = (r * r).astype(jnp.bfloat16)
        mlp_scr[...] += jnp.dot(hh, w2_ref[...], preferred_element_type=jnp.float32)

    q = q_scr[b].astype(jnp.bfloat16)
    k = k_ref[...]
    v = v_ref[...]
    s = lax.dot_general(q, k, (((1,), (1,)), ((), ())),
                        preferred_element_type=jnp.float32) * scale
    m = jnp.max(s, axis=-1, keepdims=True)
    p = jnp.exp(s - m)
    l = jnp.sum(p, axis=-1, keepdims=True)
    o = jnp.dot(p.astype(jnp.bfloat16), v, preferred_element_type=jnp.float32)
    o = o / l
    o_flat = jnp.concatenate([o[j:j + 1, :] for j in range(rep)], axis=1)
    row = lax.broadcasted_iota(jnp.int32, o_scr.shape, 0)
    o_scr[...] = jnp.where(row == b, o_flat, o_scr[...])

    @pl.when(b == n_batch - 1)
    def _oproj():
        acc_scr[...] += jnp.dot(o_scr[...].astype(jnp.bfloat16), wo_ref[...],
                                preferred_element_type=jnp.float32)

    @pl.when(step == n_steps - 1)
    def _fin():
        xf = x.astype(jnp.float32)
        gw = gw_ref[...].astype(jnp.float32)
        g = jax.nn.sigmoid(jnp.sum(xf * gw, axis=-1, keepdims=True))
        mlp = mlp_scr[...] + b2_ref[...].astype(jnp.float32)
        res = g * acc_scr[...] + (1.0 - g) * mlp
        o_ref[...] = res[:n_batch, :].astype(o_ref.dtype)


@jax.jit
def pallas_gated_mix__gqa_block_cached__dense_activation_squared_relu__decode_kernel(
    A_x: jax.Array,
    A_k_cache: jax.Array,
    A_v_cache: jax.Array,
    A_wq: jax.Array,
    A_wo: jax.Array,
    B_x: jax.Array,
    B_w1: jax.Array,
    B_b1: jax.Array,
    B_w2: jax.Array,
    B_b2: jax.Array,
    gate_w: jax.Array,
):
    del B_x
    B, Sq, D = A_x.shape
    _, Hkv, Sk, Dh = A_k_cache.shape
    Hq = A_wq.shape[1] // Dh
    rep = Hq // Hkv
    F = B_w1.shape[1]
    assert Sq == 1 and B <= _ROWS and rep <= _ROWS
    assert F % _F_CHUNK == 0
    n_fchunks = F // _F_CHUNK
    assert n_fchunks <= Hkv * B
    gw_cols = rep * Dh

    x2 = jnp.pad(A_x.reshape(B, D), ((0, _ROWS - B), (0, 0)))
    b1 = B_b1.reshape(1, F)
    b2 = B_b2.reshape(1, D)
    gw = gate_w.reshape(1, D)

    def fchunk(h, b):
        return jnp.minimum(h * B + b, n_fchunks - 1)

    kernel = functools.partial(_kernel, n_batch=B, rep=rep, dh=Dh, n_fchunks=n_fchunks)

    out = pl.pallas_call(
        kernel,
        grid=(Hkv, B),
        in_specs=[
            pl.BlockSpec((_ROWS, D), lambda h, b: (0, 0)),
            pl.BlockSpec((None, None, Sk, Dh), lambda h, b: (b, h, 0, 0)),
            pl.BlockSpec((None, None, Sk, Dh), lambda h, b: (b, h, 0, 0)),
            pl.BlockSpec((D, gw_cols), lambda h, b: (0, h)),
            pl.BlockSpec((gw_cols, D), lambda h, b: (h, 0)),
            pl.BlockSpec((D, _F_CHUNK), lambda h, b: (0, fchunk(h, b))),
            pl.BlockSpec((1, _F_CHUNK), lambda h, b: (0, fchunk(h, b))),
            pl.BlockSpec((_F_CHUNK, D), lambda h, b: (fchunk(h, b), 0)),
            pl.BlockSpec((1, D), lambda h, b: (0, 0)),
            pl.BlockSpec((1, D), lambda h, b: (0, 0)),
        ],
        out_specs=pl.BlockSpec((B, D), lambda h, b: (0, 0)),
        out_shape=jax.ShapeDtypeStruct((B, D), A_x.dtype),
        scratch_shapes=[
            pltpu.VMEM((B, _ROWS, Dh), jnp.float32),
            pltpu.VMEM((_ROWS, gw_cols), jnp.float32),
            pltpu.VMEM((_ROWS, D), jnp.float32),
            pltpu.VMEM((_ROWS, D), jnp.float32),
        ],
        compiler_params=pltpu.CompilerParams(
            dimension_semantics=("arbitrary", "arbitrary"),
            vmem_limit_bytes=64 * 1024 * 1024,
        ),
    )(x2, A_k_cache, A_v_cache, A_wq, A_wo, B_w1, b1, B_w2, b2, gw)
    return out.reshape(B, Sq, D)
```

```python
import functools

import jax
import jax.numpy as jnp
import jax.experimental.pallas as pl
import jax.experimental.pallas.tpu as pltpu
from jax import lax

_ROWS = 8
_F_CHUNK = 256


def _kernel(x_ref, k_ref, v_ref, wq_ref, wo_ref, w1_ref, b1_ref, w2_ref, b2_ref,
            gw_ref, o_ref, q_scr, o_scr, acc_scr, mlp_scr,
            *, n_batch, rep, dh, n_fchunks):
    h = pl.program_id(0)
    b = pl.program_id(1)
    step = h * n_batch + b
    n_steps = pl.num_programs(0) * pl.num_programs(1)
    scale = dh ** -0.5

    x = x_ref[...]

    @pl.when(step == 0)
    def _init():
        acc_scr[...] = jnp.zeros_like(acc_scr)
        mlp_scr[...] = jnp.zeros_like(mlp_scr)
        q_scr[...] = jnp.zeros_like(q_scr)
        o_scr[...] = jnp.zeros_like(o_scr)

    @pl.when(b == 0)
    def _qproj():
        for j in range(rep):
            qj = jnp.dot(x, wq_ref[:, j * dh:(j + 1) * dh],
                         preferred_element_type=jnp.float32)
            for bb in range(n_batch):
                q_scr[bb, j:j + 1, :] = qj[bb:bb + 1, :]

    @pl.when(step < n_fchunks)
    def _mlp():
        off = pl.multiple_of(step * _F_CHUNK, _F_CHUNK)
        b1c = b1_ref[pl.ds(off, _F_CHUNK)].astype(jnp.float32)
        hid = jnp.dot(x, w1_ref[...], preferred_element_type=jnp.float32)
        hid = hid + b1c[None, :]
        r = jnp.maximum(hid, 0.0)
        hh = (r * r).astype(jnp.bfloat16)
        mlp_scr[...] += jnp.dot(hh, w2_ref[...], preferred_element_type=jnp.float32)

    q = q_scr[b].astype(jnp.bfloat16)
    k = k_ref[...]
    v = v_ref[...]
    s = lax.dot_general(q, k, (((1,), (1,)), ((), ())),
                        preferred_element_type=jnp.float32) * scale
    m = jnp.max(s, axis=-1, keepdims=True)
    p = jnp.exp(s - m)
    l = jnp.sum(p, axis=-1, keepdims=True)
    o = jnp.dot(p.astype(jnp.bfloat16), v, preferred_element_type=jnp.float32)
    o = o / l
    o_flat = jnp.concatenate([o[j:j + 1, :] for j in range(rep)], axis=1)
    row = lax.broadcasted_iota(jnp.int32, o_scr.shape, 0)
    o_scr[...] = jnp.where(row == b, o_flat, o_scr[...])

    @pl.when(b == n_batch - 1)
    def _oproj():
        acc_scr[...] += jnp.dot(o_scr[...].astype(jnp.bfloat16), wo_ref[...],
                                preferred_element_type=jnp.float32)

    @pl.when(step == n_steps - 1)
    def _fin():
        xf = x.astype(jnp.float32)
        gw = gw_ref[...].astype(jnp.float32)
        g = jax.nn.sigmoid(jnp.sum(xf * gw[None, :], axis=-1, keepdims=True))
        mlp = mlp_scr[...] + b2_ref[...].astype(jnp.float32)[None, :]
        res = g * acc_scr[...] + (1.0 - g) * mlp
        o_ref[...] = res.astype(o_ref.dtype)


@jax.jit
def pallas_gated_mix__gqa_block_cached__dense_activation_squared_relu__decode_kernel(
    A_x, A_k_cache, A_v_cache, A_wq, A_wo, B_x, B_w1, B_b1, B_w2, B_b2, gate_w,
):
    del B_x
    B, Sq, D = A_x.shape
    _, Hkv, Sk, Dh = A_k_cache.shape
    Hq = A_wq.shape[1] // Dh
    rep = Hq // Hkv
    F = B_w1.shape[1]
    assert Sq == 1 and rep <= _ROWS
    assert F % _F_CHUNK == 0
    n_fchunks = F // _F_CHUNK
    assert n_fchunks <= Hkv * B
    gw_cols = rep * Dh

    def fchunk(h, b):
        return jnp.minimum(h * B + b, n_fchunks - 1)

    kernel = functools.partial(_kernel, n_batch=B, rep=rep, dh=Dh, n_fchunks=n_fchunks)

    out = pl.pallas_call(
        kernel,
        grid=(Hkv, B),
        in_specs=[
            pl.BlockSpec((B, D), lambda h, b: (0, 0)),
            pl.BlockSpec((None, None, Sk, Dh), lambda h, b: (b, h, 0, 0)),
            pl.BlockSpec((None, None, Sk, Dh), lambda h, b: (b, h, 0, 0)),
            pl.BlockSpec((D, gw_cols), lambda h, b: (0, h)),
            pl.BlockSpec((gw_cols, D), lambda h, b: (h, 0)),
            pl.BlockSpec((D, _F_CHUNK), lambda h, b: (0, fchunk(h, b))),
            pl.BlockSpec((F,), lambda h, b: (0,)),
            pl.BlockSpec((_F_CHUNK, D), lambda h, b: (fchunk(h, b), 0)),
            pl.BlockSpec((D,), lambda h, b: (0,)),
            pl.BlockSpec((D,), lambda h, b: (0,)),
        ],
        out_specs=pl.BlockSpec((B, D), lambda h, b: (0, 0)),
        out_shape=jax.ShapeDtypeStruct((B, D), A_x.dtype),
        scratch_shapes=[
            pltpu.VMEM((B, _ROWS, Dh), jnp.float32),
            pltpu.VMEM((B, gw_cols), jnp.float32),
            pltpu.VMEM((B, D), jnp.float32),
            pltpu.VMEM((B, D), jnp.float32),
        ],
        compiler_params=pltpu.CompilerParams(
            dimension_semantics=("arbitrary", "arbitrary"),
            vmem_limit_bytes=64 * 1024 * 1024,
        ),
    )(A_x.reshape(B, D), A_k_cache, A_v_cache, A_wq, A_wo, B_w1, B_b1, B_w2, B_b2, gate_w)
    return out.reshape(B, Sq, D)
```

```python
import functools

import jax
import jax.numpy as jnp
import jax.experimental.pallas as pl
import jax.experimental.pallas.tpu as pltpu
from jax import lax

_ROWS = 8
_NW2 = 7
_W_BACK = 2


def _kernel(x_ref, k_ref, v_ref, wq_ref, wo_ref, w1_hbm, b1_ref, w2_hbm, b2_ref,
            gw_ref, o_ref, q_scr, o_scr, acc_scr, w1_buf, w2_buf, sems,
            *, n_batch, rep, dh, w_start):
    h = pl.program_id(0)
    b = pl.program_id(1)
    step = h * n_batch + b
    n_steps = pl.num_programs(0) * pl.num_programs(1)
    scale = dh ** -0.5
    fch = w2_buf.shape[0] // _NW2

    def w1_copy():
        return pltpu.make_async_copy(w1_hbm, w1_buf, sems.at[_NW2])

    def w2_copy(c):
        return pltpu.make_async_copy(w2_hbm.at[pl.ds(c * fch, fch)],
                                     w2_buf.at[pl.ds(c * fch, fch)], sems.at[c])

    x = x_ref[...]

    @pl.when(step == 0)
    def _init():
        acc_scr[...] = jnp.zeros_like(acc_scr)
        q_scr[...] = jnp.zeros_like(q_scr)
        o_scr[...] = jnp.zeros_like(o_scr)

    @pl.when(step == w_start)
    def _start_mlp_weights():
        w1_copy().start()
        for c in range(_NW2):
            w2_copy(c).start()

    @pl.when(b == 0)
    def _qproj():
        for j in range(rep):
            qj = jnp.dot(x, wq_ref[:, j * dh:(j + 1) * dh],
                         preferred_element_type=jnp.float32)
            for bb in range(n_batch):
                q_scr[bb, j:j + 1, :] = qj[bb:bb + 1, :]

    q = q_scr[b].astype(jnp.bfloat16)
    k = k_ref[...]
    v = v_ref[...]
    s = lax.dot_general(q, k, (((1,), (1,)), ((), ())),
                        preferred_element_type=jnp.float32) * scale
    m = jnp.max(s, axis=-1, keepdims=True)
    p = jnp.exp(s - m)
    l = jnp.sum(p, axis=-1, keepdims=True)
    o = jnp.dot(p.astype(jnp.bfloat16), v, preferred_element_type=jnp.float32)
    o = o / l
    o_flat = jnp.concatenate([o[j:j + 1, :] for j in range(rep)], axis=1)
    row = lax.broadcasted_iota(jnp.int32, o_scr.shape, 0)
    o_scr[...] = jnp.where(row == b, o_flat, o_scr[...])

    @pl.when(b == n_batch - 1)
    def _oproj():
        acc_scr[...] += jnp.dot(o_scr[...].astype(jnp.bfloat16), wo_ref[...],
                                preferred_element_type=jnp.float32)

    @pl.when(step == n_steps - 1)
    def _fin():
        w1_copy().wait()
        hid = jnp.dot(x, w1_buf[...], preferred_element_type=jnp.float32)
        hid = hid + b1_ref[...].astype(jnp.float32)[None, :]
        r = jnp.maximum(hid, 0.0)
        hh = (r * r).astype(jnp.bfloat16)
        mlp = b2_ref[...].astype(jnp.float32)[None, :]
        for c in range(_NW2):
            w2_copy(c).wait()
            mlp = mlp + jnp.dot(hh[:, c * fch:(c + 1) * fch], w2_buf[pl.ds(c * fch, fch), :],
                                preferred_element_type=jnp.float32)
        xf = x.astype(jnp.float32)
        gw = gw_ref[...].astype(jnp.float32)
        g = jax.nn.sigmoid(jnp.sum(xf * gw[None, :], axis=-1, keepdims=True))
        res = g * acc_scr[...] + (1.0 - g) * mlp
        o_ref[...] = res.astype(o_ref.dtype)


@jax.jit
def pallas_gated_mix__gqa_block_cached__dense_activation_squared_relu__decode_kernel(
    A_x, A_k_cache, A_v_cache, A_wq, A_wo, B_x, B_w1, B_b1, B_w2, B_b2, gate_w,
):
    del B_x
    B, Sq, D = A_x.shape
    _, Hkv, Sk, Dh = A_k_cache.shape
    Hq = A_wq.shape[1] // Dh
    rep = Hq // Hkv
    F = B_w1.shape[1]
    assert Sq == 1 and rep <= _ROWS
    assert F % (_NW2 * 16) == 0
    gw_cols = rep * Dh

    kernel = functools.partial(_kernel, n_batch=B, rep=rep, dh=Dh,
                               w_start=max(Hkv * B - _W_BACK, 0))

    out = pl.pallas_call(
        kernel,
        grid=(Hkv, B),
        in_specs=[
            pl.BlockSpec((B, D), lambda h, b: (0, 0)),
            pl.BlockSpec((None, None, Sk, Dh), lambda h, b: (b, h, 0, 0)),
            pl.BlockSpec((None, None, Sk, Dh), lambda h, b: (b, h, 0, 0)),
            pl.BlockSpec((D, gw_cols), lambda h, b: (0, h)),
            pl.BlockSpec((gw_cols, D), lambda h, b: (h, 0)),
            pl.BlockSpec(memory_space=pl.ANY),
            pl.BlockSpec((F,), lambda h, b: (0,)),
            pl.BlockSpec(memory_space=pl.ANY),
            pl.BlockSpec((D,), lambda h, b: (0,)),
            pl.BlockSpec((D,), lambda h, b: (0,)),
        ],
        out_specs=pl.BlockSpec((B, D), lambda h, b: (0, 0)),
        out_shape=jax.ShapeDtypeStruct((B, D), A_x.dtype),
        scratch_shapes=[
            pltpu.VMEM((B, _ROWS, Dh), jnp.float32),
            pltpu.VMEM((B, gw_cols), jnp.float32),
            pltpu.VMEM((B, D), jnp.float32),
            pltpu.VMEM(B_w1.shape, B_w1.dtype),
            pltpu.VMEM(B_w2.shape, B_w2.dtype),
            pltpu.SemaphoreType.DMA((_NW2 + 1,)),
        ],
        compiler_params=pltpu.CompilerParams(
            dimension_semantics=("arbitrary", "arbitrary"),
            vmem_limit_bytes=64 * 1024 * 1024,
        ),
    )(A_x.reshape(B, D), A_k_cache, A_v_cache, A_wq, A_wo, B_w1, B_b1, B_w2, B_b2, gate_w)
    return out.reshape(B, Sq, D)
```
